```python
import os as _os
_os.environ.setdefault("JAX_PLATFORMS", "cpu")
import jax
import jax.numpy as jnp

def _softmax(x, axis=-1):
    return jax.nn.softmax(x, axis=axis)
def _gelu(x):
    return jax.nn.gelu(x, approximate=True)
def _silu(x):
    return jax.nn.silu(x)
def _sigmoid(x):
    return jax.nn.sigmoid(x)
def _layernorm(x, axis=-1, eps=1e-5):
    m = jnp.mean(x, axis=axis, keepdims=True)
    v = jnp.var(x, axis=axis, keepdims=True)
    return (x - m) / jnp.sqrt(v + eps)
def _scatter_add(tgt, idx, src, axis=0):
    return tgt.at[idx].add(src)
def _segment_sum(src, seg, n):
    return jax.ops.segment_sum(src, seg, n)
class _Rng:
    def __init__(self, key):
        self._k = key
    def _next(self):
        self._k, sub = jax.random.split(self._k)
        return sub
    def normal(self, shape):
        return jax.random.normal(self._next(), shape, dtype=jnp.bfloat16)
    def randint(self, lo, hi, shape):
        return jax.random.randint(self._next(), shape, lo, hi, dtype=jnp.int32)
    def uniform(self, shape, lo=0.0, hi=1.0):
        return jax.random.uniform(self._next(), shape, jnp.bfloat16, lo, hi)
    def permutation(self, n):
        return jax.random.permutation(self._next(), n)


kernel_name = 'standalone__se_block__vision'

def setup_inputs():
    _rng = _Rng(jax.random.key(int.from_bytes(__import__("os").urandom(4), "little")))
    _w = (lambda a: (lambda t: t.astype(jnp.bfloat16) if jnp.issubdtype(t.dtype, jnp.floating) else t)(jnp.asarray(a)))
    H = W = 384
    C = 192; r = max(C // 16, 4)
    return {
        "x": _w((lambda *s: _rng.normal(s) * 0.8)(1, H, W, C)),
        "w_down": _w((lambda *s: _rng.normal(s) * 0.8)(C, r)),
        "w_up": _w((lambda *s: _rng.normal(s) * 0.8)(r, C)),
    }

def reference(x, w_down, w_up):
    s = x.mean(axis=(1, 2))
    s = _sigmoid(_silu(s @ w_down) @ w_up)
    return x * s[:, None, None, :]
```

```python
import functools

import jax
import jax.numpy as jnp
from jax import lax
from jax.experimental import pallas as pl
from jax.experimental.pallas import tpu as pltpu

_SUB, _LANES = 8, 128
_SEG_TILES = 512
_STEP_TILES = 8
_READ_TILES = 2
_WRITE_SEGS = 6
_LOOKAHEAD = 6
_LEAD = 26
_LATE_SPLIT = 2
_LATE_BATCHES = (10, 4, 2)
_PEELED_STEPS = 2


def _tree_sum(vals):
    vals = list(vals)
    while len(vals) > 1:
        pairs = [vals[i] + vals[i + 1] for i in range(0, len(vals) - 1, 2)]
        vals = pairs + vals[2 * len(pairs):]
    return vals[0]


def _se_kernel(
    x_hbm, wd_hbm, wu_hbm, o_hbm,
    buf, wd_raw, wu_raw, wd_mxu, wd_cols, wu_cols, scale_tab,
    read_sem, late_sem, weight_sem, write_sem,
    *, lane_blocks, pixels,
):
    dtype, f32 = x_hbm.dtype, jnp.float32
    n_seg = x_hbm.shape[0]
    rank, channels = wd_hbm.shape
    groups = channels // _SUB
    phases = groups * lane_blocks // _STEP_TILES
    seg_steps = _SEG_TILES // _STEP_TILES
    cols = _STEP_TILES // _READ_TILES
    step_rows, read_rows = _STEP_TILES * _SUB, _READ_TILES * _SUB
    read_steps = n_seg // (2 * phases) * seg_steps
    read_dmas = read_steps * cols
    late_pieces = 2 * pl.cdiv(seg_steps, phases)
    step_shift, col_shift = seg_steps.bit_length() - 1, cols.bit_length() - 1
    lead_steps, lead_cols = divmod(_LEAD, cols)
    assert sum(_LATE_BATCHES) == late_pieces
    assert _LOOKAHEAD * cols + _LEAD >= late_pieces * _LATE_SPLIT

    def group_of(phase, tile):
        return (_STEP_TILES * phase + tile) // lane_blocks

    early_groups = group_of(phases - 1, 0)
    early_channels = early_groups * _SUB

    def rounded(v):
        return v.astype(dtype).astype(f32)

    def copy_in(seg, n, row, rows, sem):
        idx = (pl.ds(seg, n), pl.ds(row, rows))
        return pltpu.make_async_copy(x_hbm.at[idx], buf.at[idx], sem)

    def step_sem(queue, step):
        return read_sem.at[queue, step & (read_sem.shape[1] - 1)]

    def first_seg(queue, step):
        return ((step >> step_shift) * 2 + queue) * phases

    def start_read(k, n, queue):
        step = k >> col_shift
        row = pl.multiple_of((k & (seg_steps * cols - 1)) * read_rows, read_rows)
        copy = copy_in(first_seg(queue, step), n, row, read_rows, step_sem(queue, step))
        copy.start(priority=queue)

    def wait_step(step, n):
        row = pl.multiple_of((step & (seg_steps - 1)) * step_rows, step_rows)
        for queue in range(2):
            copy_in(first_seg(queue, step), n, row, step_rows, step_sem(queue, step)).wait()

    def is_short(step, phase):
        return (phase == 0) & (step >= read_steps - seg_steps)

    def late_piece(n):
        return n_seg - 1 - phases * (n & 1), (n >> 1) * (phases * step_rows)

    def start_late(m):
        n, rows = m >> (_LATE_SPLIT.bit_length() - 1), step_rows // _LATE_SPLIT
        seg, row = late_piece(n)
        row = pl.multiple_of(row + (m & (_LATE_SPLIT - 1)) * rows, rows)
        copy_in(seg, 1, row, rows, late_sem.at[n]).start(priority=1)

    def next_phase(step, phase):
        wrap = ((step & (seg_steps - 1)) == seg_steps - 1) | (phase == phases - 1)
        return jnp.where(wrap, 0, phase + 1)

    wd_copy = pltpu.make_async_copy(wd_hbm, wd_raw, weight_sem.at[0])
    wu_copy = pltpu.make_async_copy(wu_hbm, wu_raw, weight_sem.at[1])
    start_read(jnp.int32(0), phases, 0)
    wd_copy.start()
    wu_copy.start()

    @pl.loop(0, _LEAD + 1)
    def _(k):
        start_read(k, phases, 1)

    @pl.loop(1, _LOOKAHEAD * cols)
    def _(k):
        start_read(k, phases, 0)
        start_read(k + _LEAD, phases, 1)

    buf[n_seg, pl.ds(0, step_rows), :] = jnp.zeros((step_rows, _LANES), dtype)

    wd_copy.wait()
    wu_copy.wait()
    rank_pad = jnp.zeros((wd_mxu.shape[0] - rank, channels), f32)
    wd = jnp.concatenate([wd_raw[...].astype(f32), rank_pad], axis=0)
    wu_t = jnp.concatenate([wu_raw[...].astype(f32), rank_pad], axis=0).T
    wd_mxu[...] = wd.astype(dtype)
    for c in range(early_channels, channels):
        wd_cols[c - early_channels] = jnp.broadcast_to(wd[:, c:c + 1], wd_cols.shape[1:])
    for j in range(rank):
        wu_cols[j] = jnp.broadcast_to(wu_t[:, j:j + 1], wu_cols.shape[1:])

    def accumulate(acc, pieces):
        terms = [[] for _ in acc]
        for phase, seg, row in pieces:
            v = buf[seg, pl.ds(row, step_rows), :].astype(f32)
            for t in range(_STEP_TILES):
                terms[group_of(phase, t)].append(v[_SUB * t:_SUB * (t + 1)])
        return tuple(_tree_sum(new + [old]) for new, old in zip(terms, acc))

    def read_step(step, carry):
        phase, phase0, phase1, acc = carry
        step0, step1 = step + _LOOKAHEAD, step + _LOOKAHEAD + lead_steps
        phase2 = next_phase(step1, phase1)
        short, short0 = is_short(step, phase), is_short(step0, phase0)
        for c in range(cols):
            k0 = step0 * cols + c
            k1 = k0 + _LEAD
            if c + lead_cols < cols:
                short1 = is_short(step1, phase1)
            else:
                short1 = is_short(step1 + 1, phase2)
            for k, is_cut, queue in ((k0, short0, 0), (k1, short1, 1)):
                pl.when((k < read_dmas) & ~is_cut)(
                    functools.partial(start_read, k, phases, queue))
                pl.when((k < read_dmas) & is_cut)(
                    functools.partial(start_read, k, phases - 1, queue))
            pl.when((k1 >= read_dmas) & (k1 < read_dmas + late_pieces * _LATE_SPLIT))(
                functools.partial(start_late, k1 - read_dmas))
        pl.when(~short)(functools.partial(wait_step, step, phases))
        pl.when(short)(functools.partial(wait_step, step, phases - 1))

        row = pl.multiple_of((step & (seg_steps - 1)) * step_rows, step_rows)
        pieces = []
        for p in range(phases):
            k = jnp.where(p >= phase, p - phase, p - phase + phases)
            for queue in range(2):
                seg = first_seg(queue, step) + k
                if p == phases - 1:
                    pieces.append((
                        p,
                        jnp.where(short, n_seg, seg),
                        pl.multiple_of(jnp.where(short, 0, row), step_rows),
                    ))
                else:
                    pieces.append((p, seg, row))
        return next_phase(step, phase), next_phase(step0, phase0), phase2, accumulate(acc, pieces)

    acc = lax.fori_loop(
        0,
        read_steps,
        read_step,
        (
            jnp.int32(0),
            jnp.int32(_LOOKAHEAD % phases),
            jnp.int32((_LOOKAHEAD + lead_steps) % phases),
            tuple(jnp.zeros((_SUB, _LANES), f32) for _ in range(groups)),
        ),
    )[-1]

    def means(sums):
        m = jnp.sum(jnp.concatenate(sums, axis=0), axis=1, keepdims=True) * (1.0 / pixels)
        return jnp.broadcast_to(m, (_SUB * len(sums), _LANES)).astype(dtype)

    z_early = jnp.dot(
        wd_mxu[:, :early_channels], means(acc[:early_groups]), preferred_element_type=f32)
    done = 0
    for count in _LATE_BATCHES:
        batch = range(done, done + count)
        for n in batch:
            seg, row = late_piece(n)
            copy_in(seg, 1, row, step_rows, late_sem.at[n]).wait()
        acc = accumulate(acc, [(phases - 1, *late_piece(n)) for n in batch])
        done += count
    m_late = means(acc[early_groups:]).astype(f32)
    z = rounded(_tree_sum(
        [
            wd_cols[c] * jnp.broadcast_to(m_late[c:c + 1], wd_cols.shape[1:])
            for c in range(channels - early_channels)
        ]
        + [z_early]
    ))
    h = rounded(z * jax.nn.sigmoid(z))
    h_rows = [jnp.broadcast_to(h[j:j + 1], (_SUB, _LANES)) for j in range(rank)]

    gates = {}

    def gate(g):
        if g not in gates:
            y = _tree_sum(
                [wu_cols[j, pl.ds(g * _SUB, _SUB), :] * h_rows[j] for j in range(rank)])
            gates[g] = rounded(jax.nn.sigmoid(rounded(y)))
        return gates[g]

    def phase_scale(phase):
        return jnp.concatenate([gate(group_of(phase, t)) for t in range(_STEP_TILES)], axis=0)

    def scale_piece(seg, rows, scale):
        buf[seg, rows, :] = (buf[seg, rows, :].astype(f32) * scale).astype(dtype)

    for step in range(_PEELED_STEPS):
        rows = pl.ds(step * step_rows, step_rows)
        for seg in range(_WRITE_SEGS):
            scale_piece(seg, rows, phase_scale((seg + step) % phases))
            pltpu.make_async_copy(buf.at[seg, rows], o_hbm.at[seg, rows], write_sem).start()
    for phase in range(phases):
        scale_tab[phase] = phase_scale(phase)

    def write_step(step, phase):
        seg0, pos = (step >> step_shift) * _WRITE_SEGS, step & (seg_steps - 1)
        rows = pl.ds(pl.multiple_of(pos * step_rows, step_rows), step_rows)
        for k in range(_WRITE_SEGS):
            p = jnp.where(phase + k >= phases, phase + k - phases, phase + k)
            scale_piece(seg0 + k, rows, scale_tab[p])
        idx = (pl.ds(seg0, _WRITE_SEGS), rows)
        pltpu.make_async_copy(buf.at[idx], o_hbm.at[idx], write_sem).start()
        phase += jnp.where(pos == seg_steps - 1, (_WRITE_SEGS - seg_steps + 1) % phases, 1)
        return jnp.where(phase >= phases, phase - phases, phase)

    lax.fori_loop(
        _PEELED_STEPS,
        n_seg // _WRITE_SEGS * seg_steps,
        write_step,
        jnp.int32(_PEELED_STEPS % phases),
    )
    pltpu.make_async_copy(buf.at[pl.ds(0, n_seg)], o_hbm, write_sem).wait()


@jax.jit
def pallas_standalone__se_block__vision_kernel(
    x: jax.Array,
    w_down: jax.Array,
    w_up: jax.Array,
):
    batch, height, width, channels = x.shape
    rank = w_down.shape[1]
    groups, lane_blocks = channels // _SUB, width // _LANES
    row_tiles = groups * lane_blocks
    phases = row_tiles // _STEP_TILES
    n_seg = height * row_tiles // _SEG_TILES
    seg_rows = _SEG_TILES * _SUB
    assert batch == 1 and channels % _SUB == 0 and width % _LANES == 0
    assert n_seg * _SEG_TILES == height * row_tiles
    assert row_tiles % _STEP_TILES == 0 and _SEG_TILES % row_tiles == _STEP_TILES
    assert n_seg % (2 * phases) == 0 and n_seg % _WRITE_SEGS == 0 and _WRITE_SEGS <= phases
    rank_rows = pl.cdiv(rank, 16) * 16
    late_channels = channels - (row_tiles - _STEP_TILES) // lane_blocks * _SUB
    steps_in_flight = _LOOKAHEAD + _LEAD * _READ_TILES // _STEP_TILES + 2

    tiles = jnp.transpose(x, (0, 1, 3, 2)).reshape(height, groups, _SUB, lane_blocks, _LANES)
    tiles = jnp.transpose(tiles, (0, 1, 3, 2, 4)).reshape(n_seg, seg_rows, _LANES)

    hbm = pl.BlockSpec(memory_space=pltpu.MemorySpace.HBM)
    out = pl.pallas_call(
        functools.partial(_se_kernel, lane_blocks=lane_blocks, pixels=height * width),
        in_specs=[hbm, hbm, hbm],
        out_specs=hbm,
        out_shape=jax.ShapeDtypeStruct(tiles.shape, x.dtype),
        scratch_shapes=[
            pltpu.VMEM((n_seg + 1, seg_rows, _LANES), x.dtype),
            pltpu.VMEM((rank, channels), w_down.dtype),
            pltpu.VMEM((rank, channels), w_up.dtype),
            pltpu.VMEM((rank_rows, channels), x.dtype),
            pltpu.VMEM((late_channels, rank_rows, _LANES), jnp.float32),
            pltpu.VMEM((rank, channels, _LANES), jnp.float32),
            pltpu.VMEM((phases, _STEP_TILES * _SUB, _LANES), jnp.float32),
            pltpu.SemaphoreType.DMA((2, 1 << steps_in_flight.bit_length())),
            pltpu.SemaphoreType.DMA((sum(_LATE_BATCHES),)),
            pltpu.SemaphoreType.DMA((2,)),
            pltpu.SemaphoreType.DMA(()),
        ],
        compiler_params=pltpu.CompilerParams(
            vmem_limit_bytes=100 * 1024 * 1024,
            disable_bounds_checks=True,
            disable_semaphore_checks=True,
        ),
        name="se_block",
    )(tiles, w_down.T, w_up)

    out = out.reshape(height, groups, lane_blocks, _SUB, _LANES)
    out = jnp.transpose(out, (0, 1, 3, 2, 4)).reshape(batch, height, channels, width)
    return jnp.transpose(out, (0, 1, 3, 2))
```

```python
import functools

import jax
import jax.numpy as jnp
import numpy as np
from jax import lax
from jax.experimental import pallas as pl
from jax.experimental.pallas import tpu as pltpu

_SUB, _LANES = 8, 128
_SEG_TILES = 512
_STEP_TILES = 8
_READ_SEGS = (2, 2, 2, 2, 1)
_WRITE_SEGS = 6
_LOOKAHEAD = 6
_LEAD = 5
_LATE_SPLIT = 2
_LATE_BATCHES = (10, 4, 2)
_PEELED_STEPS = 2


def _tree_sum(vals):
    vals = list(vals)
    while len(vals) > 1:
        pairs = [vals[i] + vals[i + 1] for i in range(0, len(vals) - 1, 2)]
        vals = pairs + vals[2 * len(pairs):]
    return vals[0]


def _se_kernel(
    x_hbm, wd_hbm, wu_hbm, o_hbm,
    buf, wd_raw, wu_raw, wd_mxu, wd_cols, wu_cols, scale_tab,
    read_sem, late_sem, weight_sem, write_sem,
    *, lane_blocks, pixels,
):
    dtype, f32 = x_hbm.dtype, jnp.float32
    n_seg = x_hbm.shape[0]
    rank, channels = wd_hbm.shape
    groups = channels // _SUB
    phases = groups * lane_blocks // _STEP_TILES
    seg_steps = _SEG_TILES // _STEP_TILES
    cols = len(_READ_SEGS)
    step_rows = _STEP_TILES * _SUB
    read_steps = n_seg // (2 * phases) * seg_steps
    late_pieces = 2 * pl.cdiv(seg_steps, phases)
    late_dmas = late_pieces * _LATE_SPLIT
    step_shift = seg_steps.bit_length() - 1
    assert sum(_READ_SEGS) == phases and _READ_SEGS[-1] == 1
    assert sum(_LATE_BATCHES) == late_pieces
    assert (_LOOKAHEAD + _LEAD) * cols >= late_dmas

    def group_of(phase, tile):
        return (_STEP_TILES * phase + tile) // lane_blocks

    early_groups = group_of(phases - 1, 0)
    early_channels = early_groups * _SUB

    def rounded(v):
        return v.astype(dtype).astype(f32)

    def copy_in(seg, n, row, rows, sem):
        idx = (pl.ds(seg, n), pl.ds(row, rows))
        return pltpu.make_async_copy(x_hbm.at[idx], buf.at[idx], sem)

    def step_sem(queue, step):
        return read_sem.at[queue, step & (read_sem.shape[1] - 1)]

    def first_seg(queue, step):
        return ((step >> step_shift) * 2 + queue) * phases

    def start_read(step, col, queue):
        row = pl.multiple_of((step & (seg_steps - 1)) * step_rows, step_rows)
        seg = first_seg(queue, step) + sum(_READ_SEGS[:col])
        copy = copy_in(seg, _READ_SEGS[col], row, step_rows, step_sem(queue, step))
        copy.start(priority=queue)

    def wait_step(step, n):
        row = pl.multiple_of((step & (seg_steps - 1)) * step_rows, step_rows)
        for queue in range(2):
            copy_in(first_seg(queue, step), n, row, step_rows, step_sem(queue, step)).wait()

    def is_short(step, phase):
        return (phase == 0) & (step >= read_steps - seg_steps)

    def late_piece(n):
        return n_seg - 1 - phases * (n & 1), (n >> 1) * (phases * step_rows)

    def start_late(m):
        n, rows = m >> (_LATE_SPLIT.bit_length() - 1), step_rows // _LATE_SPLIT
        seg, row = late_piece(n)
        row = pl.multiple_of(row + (m & (_LATE_SPLIT - 1)) * rows, rows)
        copy_in(seg, 1, row, rows, late_sem.at[n]).start(priority=1)

    def next_phase(step, phase):
        wrap = ((step & (seg_steps - 1)) == seg_steps - 1) | (phase == phases - 1)
        return jnp.where(wrap, 0, phase + 1)

    wd_copy = pltpu.make_async_copy(wd_hbm, wd_raw, weight_sem.at[0])
    wu_copy = pltpu.make_async_copy(wu_hbm, wu_raw, weight_sem.at[1])
    start_read(np.int32(0), 0, 0)
    wd_copy.start()
    wu_copy.start()

    @pl.loop(0, _LEAD)
    def _(step):
        for col in range(cols):
            start_read(step, col, 1)

    @pl.loop(0, _LOOKAHEAD)
    def _(step):
        pl.when(step > 0)(functools.partial(start_read, step, 0, 0))
        start_read(step + _LEAD, 0, 1)
        for col in range(1, cols):
            start_read(step, col, 0)
            start_read(step + _LEAD, col, 1)

    buf[n_seg, pl.ds(0, step_rows), :] = jnp.zeros((step_rows, _LANES), dtype)

    wd_copy.wait()
    wu_copy.wait()
    rank_pad = jnp.zeros((wd_mxu.shape[0] - rank, channels), f32)
    wd = jnp.concatenate([wd_raw[...].astype(f32), rank_pad], axis=0)
    wu_t = jnp.concatenate([wu_raw[...].astype(f32), rank_pad], axis=0).T
    wd_mxu[...] = wd.astype(dtype)
    for c in range(early_channels, channels):
        wd_cols[c - early_channels] = jnp.broadcast_to(wd[:, c:c + 1], wd_cols.shape[1:])
    for j in range(rank):
        wu_cols[j] = jnp.broadcast_to(wu_t[:, j:j + 1], wu_cols.shape[1:])

    def accumulate(acc, pieces):
        terms = [[] for _ in acc]
        for phase, seg, row in pieces:
            v = buf[seg, pl.ds(row, step_rows), :].astype(f32)
            for t in range(_STEP_TILES):
                terms[group_of(phase, t)].append(v[_SUB * t:_SUB * (t + 1)])
        return tuple(_tree_sum(new + [old]) for new, old in zip(terms, acc))

    def read_step(step, carry):
        phase, phase0, phase1, acc = carry
        step0, step1 = step + _LOOKAHEAD, step + _LOOKAHEAD + _LEAD
        for col in range(cols):
            for queue, (ahead, ahead_phase) in enumerate(((step0, phase0), (step1, phase1))):
                go = ahead < read_steps
                if col == cols - 1:
                    go &= ~is_short(ahead, ahead_phase)
                pl.when(go)(functools.partial(start_read, ahead, col, queue))
            late = (step1 - read_steps) * cols + col
            pl.when((late >= 0) & (late < late_dmas))(functools.partial(start_late, late))
        short = is_short(step, phase)
        pl.when(~short)(functools.partial(wait_step, step, phases))
        pl.when(short)(functools.partial(wait_step, step, phases - 1))

        row = pl.multiple_of((step & (seg_steps - 1)) * step_rows, step_rows)
        pieces = []
        for p in range(phases):
            k = jnp.where(p >= phase, p - phase, p - phase + phases)
            for queue in range(2):
                seg = first_seg(queue, step) + k
                if p == phases - 1:
                    pieces.append((
                        p,
                        jnp.where(short, n_seg, seg),
                        pl.multiple_of(jnp.where(short, 0, row), step_rows),
                    ))
                else:
                    pieces.append((p, seg, row))
        return (
            next_phase(step, phase),
            next_phase(step0, phase0),
            next_phase(step1, phase1),
            accumulate(acc, pieces),
        )

    acc = lax.fori_loop(
        0,
        read_steps,
        read_step,
        (
            np.int32(0),
            np.int32(_LOOKAHEAD % phases),
            np.int32((_LOOKAHEAD + _LEAD) % phases),
            tuple(jnp.zeros((_SUB, _LANES), f32) for _ in range(groups)),
        ),
    )[-1]

    def means(sums):
        m = jnp.sum(jnp.concatenate(sums, axis=0), axis=1, keepdims=True) * (1.0 / pixels)
        return jnp.broadcast_to(m, (_SUB * len(sums), _LANES)).astype(dtype)

    z_early = jnp.dot(
        wd_mxu[:, :early_channels], means(acc[:early_groups]), preferred_element_type=f32)
    done = 0
    for count in _LATE_BATCHES:
        batch = range(done, done + count)
        for n in batch:
            seg, row = late_piece(n)
            copy_in(seg, 1, row, step_rows, late_sem.at[n]).wait()
        acc = accumulate(acc, [(phases - 1, *late_piece(n)) for n in batch])
        done += count
    m_late = means(acc[early_groups:]).astype(f32)
    z = rounded(_tree_sum(
        [
            wd_cols[c] * jnp.broadcast_to(m_late[c:c + 1], wd_cols.shape[1:])
            for c in range(channels - early_channels)
        ]
        + [z_early]
    ))
    h = rounded(z * jax.nn.sigmoid(z))
    h_rows = [jnp.broadcast_to(h[j:j + 1], (_SUB, _LANES)) for j in range(rank)]

    gates = {}

    def gate(g):
        if g not in gates:
            y = _tree_sum(
                [wu_cols[j, pl.ds(g * _SUB, _SUB), :] * h_rows[j] for j in range(rank)])
            gates[g] = rounded(jax.nn.sigmoid(rounded(y)))
        return gates[g]

    def phase_scale(phase):
        return jnp.concatenate([gate(group_of(phase, t)) for t in range(_STEP_TILES)], axis=0)

    def scale_piece(seg, rows, scale):
        buf[seg, rows, :] = (buf[seg, rows, :].astype(f32) * scale).astype(dtype)

    for step in range(_PEELED_STEPS):
        rows = pl.ds(step * step_rows, step_rows)
        for seg in range(_WRITE_SEGS):
            scale_piece(seg, rows, phase_scale((seg + step) % phases))
            pltpu.make_async_copy(buf.at[seg, rows], o_hbm.at[seg, rows], write_sem).start()
    for phase in range(phases):
        scale_tab[phase] = phase_scale(phase)

    def write_step(step, phase):
        seg0, pos = (step >> step_shift) * _WRITE_SEGS, step & (seg_steps - 1)
        rows = pl.ds(pl.multiple_of(pos * step_rows, step_rows), step_rows)
        for k in range(_WRITE_SEGS):
            p = jnp.where(phase + k >= phases, phase + k - phases, phase + k)
            scale_piece(seg0 + k, rows, scale_tab[p])
        idx = (pl.ds(seg0, _WRITE_SEGS), rows)
        pltpu.make_async_copy(buf.at[idx], o_hbm.at[idx], write_sem).start()
        phase += jnp.where(pos == seg_steps - 1, (_WRITE_SEGS - seg_steps + 1) % phases, 1)
        return jnp.where(phase >= phases, phase - phases, phase)

    lax.fori_loop(
        _PEELED_STEPS,
        n_seg // _WRITE_SEGS * seg_steps,
        write_step,
        np.int32(_PEELED_STEPS % phases),
    )
    pltpu.make_async_copy(buf.at[pl.ds(0, n_seg)], o_hbm, write_sem).wait()


@jax.jit
def pallas_standalone__se_block__vision_kernel(
    x: jax.Array,
    w_down: jax.Array,
    w_up: jax.Array,
):
    batch, height, width, channels = x.shape
    rank = w_down.shape[1]
    groups, lane_blocks = channels // _SUB, width // _LANES
    row_tiles = groups * lane_blocks
    phases = row_tiles // _STEP_TILES
    n_seg = height * row_tiles // _SEG_TILES
    seg_rows = _SEG_TILES * _SUB
    assert batch == 1 and channels % _SUB == 0 and width % _LANES == 0
    assert n_seg * _SEG_TILES == height * row_tiles
    assert row_tiles % _STEP_TILES == 0 and _SEG_TILES % row_tiles == _STEP_TILES
    assert n_seg % (2 * phases) == 0 and n_seg % _WRITE_SEGS == 0 and _WRITE_SEGS <= phases
    rank_rows = pl.cdiv(rank, 16) * 16
    late_channels = channels - (row_tiles - _STEP_TILES) // lane_blocks * _SUB
    steps_in_flight = _LOOKAHEAD + _LEAD + 1

    tiles = jnp.transpose(x, (0, 1, 3, 2)).reshape(height, groups, _SUB, lane_blocks, _LANES)
    tiles = jnp.transpose(tiles, (0, 1, 3, 2, 4)).reshape(n_seg, seg_rows, _LANES)

    hbm = pl.BlockSpec(memory_space=pltpu.MemorySpace.HBM)
    out = pl.pallas_call(
        functools.partial(_se_kernel, lane_blocks=lane_blocks, pixels=height * width),
        in_specs=[hbm, hbm, hbm],
        out_specs=hbm,
        out_shape=jax.ShapeDtypeStruct(tiles.shape, x.dtype),
        scratch_shapes=[
            pltpu.VMEM((n_seg + 1, seg_rows, _LANES), x.dtype),
            pltpu.VMEM((rank, channels), w_down.dtype),
            pltpu.VMEM((rank, channels), w_up.dtype),
            pltpu.VMEM((rank_rows, channels), x.dtype),
            pltpu.VMEM((late_channels, rank_rows, _LANES), jnp.float32),
            pltpu.VMEM((rank, channels, _LANES), jnp.float32),
            pltpu.VMEM((phases, _STEP_TILES * _SUB, _LANES), jnp.float32),
            pltpu.SemaphoreType.DMA((2, 1 << steps_in_flight.bit_length())),
            pltpu.SemaphoreType.DMA((sum(_LATE_BATCHES),)),
            pltpu.SemaphoreType.DMA((2,)),
            pltpu.SemaphoreType.DMA(()),
        ],
        compiler_params=pltpu.CompilerParams(
            vmem_limit_bytes=100 * 1024 * 1024,
            disable_bounds_checks=True,
            disable_semaphore_checks=True,
        ),
        name="se_block",
    )(tiles, w_down.T, w_up)

    out = out.reshape(height, groups, lane_blocks, _SUB, _LANES)
    out = jnp.transpose(out, (0, 1, 3, 2, 4)).reshape(batch, height, channels, width)
    return jnp.transpose(out, (0, 1, 3, 2))
```
